```python
import jax
import jax.numpy as jnp

def _softmax(x, axis=-1):
    return jax.nn.softmax(x, axis=axis)

def _gelu(x):
    return jax.nn.gelu(x, approximate=True)

def _silu(x):
    return jax.nn.silu(x)

def _sigmoid(x):
    return jax.nn.sigmoid(x)

def _layernorm(x, axis=-1, eps=1e-05):
    m = jnp.mean(x, axis=axis, keepdims=True)
    v = jnp.var(x, axis=axis, keepdims=True)
    return (x - m) / jnp.sqrt(v + eps)

def _scatter_add(tgt, idx, src, axis=0):
    return tgt.at[idx].add(src)

def _segment_sum(src, seg, n):
    return jax.ops.segment_sum(src, seg, n)

class _Rng:

    def __init__(self, key):
        self._k = key

    def _next(self):
        self._k, sub = jax.random.split(self._k)
        return sub

    def normal(self, shape):
        return jax.random.normal(self._next(), shape, dtype=jnp.bfloat16)

    def randint(self, lo, hi, shape):
        return jax.random.randint(self._next(), shape, lo, hi, dtype=jnp.int32)

    def uniform(self, shape, lo=0.0, hi=1.0):
        return jax.random.uniform(self._next(), shape, jnp.bfloat16, lo, hi)

    def permutation(self, n):
        return jax.random.permutation(self._next(), n)
kernel_name = 'adaLN_cond__gqa_block_cached__moe_arch_mod__prompt'

def setup_inputs():
    _rng = _Rng(jax.random.key(int.from_bytes(__import__("os").urandom(4), "little")))
    _w = lambda a: (lambda t: t.astype(jnp.bfloat16) if jnp.issubdtype(t.dtype, jnp.floating) else t)(jnp.asarray(a))

    def _A_setup():
        B, Sq, D = (1, 2048, 576)
        Hq, Hkv, Sk, Dh = (32, 16, 2048, 128)
        assert Hq % Hkv == 0, (Hq, Hkv)
        return {'x': _w((lambda *s: _rng.normal(s) * 0.05)(B, Sq, D)), 'k_cache': _w((lambda *s: _rng.normal(s) * 0.05)(B, Hkv, Sk, Dh)), 'v_cache': _w((lambda *s: _rng.normal(s) * 0.05)(B, Hkv, Sk, Dh)), 'wq': _w((lambda *s: _rng.normal(s) * 0.05)(D, Hq * Dh) * D ** (-0.5)), 'wo': _w((lambda *s: _rng.normal(s) * 0.05)(Hq * Dh, D) * (Hq * Dh) ** (-0.5))}
    _A_in = _A_setup()

    def _B_setup():
        B, S, D, F, C = (1, 2048, 576, 4608, 8)
        return {'x': _w((lambda *s: _rng.normal(s) * 0.05)(B, S, D)), 'w_r': _w((lambda *s: _rng.normal(s) * 0.05)(D)), 'w_gate': _w((lambda *s: _rng.normal(s) * 0.05)(D, F)), 'w_up': _w((lambda *s: _rng.normal(s) * 0.05)(D, F)), 'w_down': _w((lambda *s: _rng.normal(s) * 0.05)(F, D))}
    _B_in = _B_setup()
    return {'A_x': _A_in['x'], 'A_k_cache': _A_in['k_cache'], 'A_v_cache': _A_in['v_cache'], 'A_wq': _A_in['wq'], 'A_wo': _A_in['wo'], 'B_x': _B_in['x'], 'B_w_r': _B_in['w_r'], 'B_w_gate': _B_in['w_gate'], 'B_w_up': _B_in['w_up'], 'B_w_down': _B_in['w_down'], 'c': _w((lambda *s: _rng.normal(s) * 0.05)(1, 576)), 'w_mod': _w((lambda *s: _rng.normal(s) * 0.05)(576, 6 * 576) * 576 ** (-0.5))}

def reference(A_x, A_k_cache, A_v_cache, A_wq, A_wo, B_x, B_w_r, B_w_gate, B_w_up, B_w_down, c, w_mod):

    def _A_ref(x, k_cache, v_cache, wq, wo):
        B, Sq, D = x.shape
        Hq, Dh = (32, 128)
        Hkv = k_cache.shape[1]
        rep = Hq // Hkv
        q = (lambda x, *d: x.transpose(*d))((x @ wq).reshape(B, Sq, Hq, Dh), 0, 2, 1, 3)
        k = jnp.repeat(k_cache, rep, axis=1)
        v = jnp.repeat(v_cache, rep, axis=1)
        scores = jnp.einsum('bhqd,bhkd->bhqk', q, k) * Dh ** (-0.5)
        p = _softmax(scores, axis=-1)
        o = jnp.einsum('bhqk,bhkd->bhqd', p, v)
        return (lambda x, *d: x.transpose(*d))(o, 0, 2, 1, 3).reshape(B, Sq, Hq * Dh) @ wo

    def _B_ref(x, w_r, w_gate, w_up, w_down):
        B, S, D = x.shape
        C = 8
        r = x @ w_r
        idx = jnp.argsort(-r, axis=-1)[:, :C]
        idx_e = jnp.repeat(idx.reshape(B, C, 1), D, axis=2)
        x_sel = jnp.take_along_axis(x, idx_e, axis=1)
        g = _silu(x_sel @ w_gate)
        u = x_sel @ w_up
        y = g * u @ w_down
        r_sel = _sigmoid(jnp.take_along_axis(r, idx, axis=1))
        y = y * r_sel.reshape(B, C, 1)
        b_off = (jnp.arange(B) * S).reshape(B, 1)
        flat_idx = (idx + b_off).reshape(B * C)
        zero = (x * 0.0).reshape(B * S, D)
        upd = _scatter_add(zero, flat_idx, y.reshape(B * C, D), axis=0)
        return x + upd.reshape(B, S, D)
    x = A_x
    mod = (_silu(c) @ w_mod).reshape(c.shape[0], 6, 1, -1)
    sa, ca, ga, sb, cb, gb = (mod[:, 0].copy(), mod[:, 1].copy(), mod[:, 2].copy(), mod[:, 3].copy(), mod[:, 4].copy(), mod[:, 5].copy())
    h = _layernorm(x, axis=-1) * (1 + ca) + sa
    x = x + ga * _A_ref(h, A_k_cache, A_v_cache, A_wq, A_wo)
    h = _layernorm(x, axis=-1) * (1 + cb) + sb
    x = x + gb * _B_ref(h, B_w_r, B_w_gate, B_w_up, B_w_down)
    return x
```

```python
import jax
import jax.numpy as jnp
from jax import lax
import jax.experimental.pallas as pl
import jax.experimental.pallas.tpu as pltpu

S = 2048
D = 576
HQ, HKV, DH = 32, 16, 128
SK = 2048
F = 4608
C = 8

BF = jnp.bfloat16
F32 = jnp.float32
U32 = jnp.uint32
NT = (((1,), (1,)), ((), ()))

LOG2E = 1.4426950408889634
QSCALE = (DH ** -0.5) * LOG2E
EPS_BF = 1.0013580322265625e-05

R1 = 256
RA = 128
CK = 512
R3 = 256
NQ = 512


def _b(x):
    return x.astype(BF).astype(F32)


def _ln_mod_t(x, one_c, s):
    mean = jnp.sum(x, axis=0, keepdims=True) * (1.0 / D)
    xc = x - mean
    var = jnp.sum(xc * xc, axis=0, keepdims=True) * (1.0 / D)
    sq = _b(jnp.sqrt(_b(_b(var) + EPS_BF)))
    inv = 1.0 / sq
    hn = _b(_b(x - _b(mean)) * inv)
    return _b(_b(hn * one_c) + s)


def _sigmoid_b(x):
    return _b(1.0 / _b(1.0 + _b(jnp.exp(-x))))


def _cols(row):
    return jnp.broadcast_to(row, (128, row.shape[1])).T


def _tile_lanes(ref, n):
    v = ref[...]
    return jnp.concatenate([v] * n, axis=1) if n > 1 else v


def _kernel(x_hbm, k_hbm, v_hbm, wq_hbm, wo_hbm, wr_ref, wg_hbm, wu_hbm, wd_hbm, c_ref, wm_hbm,
            out_hbm,
            x_v, k_v, v_v, wq_v, wo_v, wg_v, wu_v, wd_v, wm_v, q_v, o_v, out_v,
            sa_v, ca_v, ga_v, sb_v, cb_v, gb_v, wr_v, sems):
    nx = S // R1
    nq = (HQ * DH) // NQ

    cp_wma = pltpu.make_async_copy(wm_hbm.at[:, pl.ds(0, 2 * D)], wm_v.at[:, pl.ds(0, 2 * D)], sems.at[0])
    cp_x = [pltpu.make_async_copy(x_hbm.at[0, :, pl.ds(i * R1, R1)], x_v.at[:, pl.ds(i * R1, R1)], sems.at[1 + i])
            for i in range(nx)]
    cp_wq = [pltpu.make_async_copy(wq_hbm.at[:, pl.ds(i * NQ, NQ)], wq_v.at[:, pl.ds(i * NQ, NQ)], sems.at[1 + nx + i])
             for i in range(nq)]
    base = 1 + nx + nq
    cp_k = pltpu.make_async_copy(k_hbm.at[0], k_v, sems.at[base])
    cp_v = pltpu.make_async_copy(v_hbm.at[0], v_v, sems.at[base + 1])
    cp_wo = pltpu.make_async_copy(wo_hbm, wo_v, sems.at[base + 2])
    cp_wmb = pltpu.make_async_copy(wm_hbm.at[:, pl.ds(2 * D, 4 * D)], wm_v.at[:, pl.ds(2 * D, 4 * D)], sems.at[base + 3])
    cp_wg = pltpu.make_async_copy(wg_hbm, wg_v, sems.at[base + 4])
    cp_wu = pltpu.make_async_copy(wu_hbm, wu_v, sems.at[base + 5])
    cp_wd = pltpu.make_async_copy(wd_hbm, wd_v, sems.at[base + 6])
    cp_out = pltpu.make_async_copy(out_v, out_hbm.at[0], sems.at[base + 7])

    cp_wma.start()
    cp_x[0].start()
    for cp in cp_wq:
        cp.start()
    for cp in cp_x[1:]:
        cp.start()

    c = c_ref[...].astype(F32)
    sc = _b(c * _sigmoid_b(c)).astype(BF)
    sc8 = jnp.broadcast_to(sc, (8, D))
    cp_wma.wait()
    moda = _b(jnp.dot(sc8, wm_v[:, 0:2 * D], preferred_element_type=F32))[0:1]
    moda_c = _cols(moda)
    sa_v[...] = moda_c[0:D]
    ca_v[...] = _b(1.0 + moda_c[D:2 * D])

    for t in range(nx):
        cp_x[t].wait()
        xt = x_v[:, t * R1:(t + 1) * R1].astype(F32)
        ht = _ln_mod_t(xt, _tile_lanes(ca_v, R1 // 128), _tile_lanes(sa_v, R1 // 128))
        h = ht.T.astype(BF)
        for n in range(nq):
            if t == 0:
                cp_wq[n].wait()
                if n == nq - 1:
                    cp_k.start(); cp_v.start(); cp_wo.start(); cp_wmb.start()
                    cp_wg.start(); cp_wu.start(); cp_wd.start()
            qn = jnp.dot(h, wq_v[:, n * NQ:(n + 1) * NQ], preferred_element_type=F32) * QSCALE
            for i in range(NQ // DH):
                q_v[n * (NQ // DH) + i, t * R1:(t + 1) * R1, :] = qn[:, i * DH:(i + 1) * DH].astype(BF)

    cp_k.wait()
    cp_v.wait()
    nck = SK // CK
    rep = HQ // HKV

    def attn_body(g, carry):
        tiles = [(hh, t) for hh in range(rep) for t in range(S // RA)]
        steps = [(ti, j) for ti in range(len(tiles)) for j in range(nck)]

        def qk(ti, j):
            hh, t = tiles[ti]
            q = q_v[g * rep + hh, t * RA:(t + 1) * RA, :]
            return lax.dot_general(q, k_v[g, j * CK:(j + 1) * CK, :], NT, preferred_element_type=F32)

        s = qk(0, 0)
        m = l = acc = None
        for n, (ti, j) in enumerate(steps):
            s_next = qk(*steps[n + 1]) if n + 1 < len(steps) else None
            cm = s[:, 0:128]
            for i in range(1, CK // 128):
                cm = jnp.maximum(cm, s[:, i * 128:(i + 1) * 128])
            cm = jnp.max(cm, axis=1, keepdims=True)
            if m is None:
                m_new, alpha = cm, None
            else:
                m_new = jnp.maximum(m, cm)
                alpha = jnp.exp2(m - m_new)
            p = jnp.exp2(s - m_new)
            ls = p[:, 0:128]
            for i in range(1, CK // 128):
                ls = ls + p[:, i * 128:(i + 1) * 128]
            l = ls if l is None else alpha * l + ls
            o = jnp.dot(p.astype(BF), v_v[g, j * CK:(j + 1) * CK, :], preferred_element_type=F32)
            acc = o if acc is None else alpha * acc + o
            m = m_new
            if j == nck - 1:
                hh, t = tiles[ti]
                lsum = jnp.sum(l, axis=1, keepdims=True)
                rl = pl.reciprocal(lsum, approx=True)
                rl = rl * (2.0 - lsum * rl)
                o_v[g * rep + hh, t * RA:(t + 1) * RA, :] = (acc * rl).astype(BF)
                m = l = acc = None
            s = s_next
        return carry

    lax.fori_loop(0, HKV, attn_body, 0)

    cp_wmb.wait()
    modb = _b(jnp.dot(sc8, wm_v[:, 2 * D:6 * D], preferred_element_type=F32))[0:1]
    modb_c = _cols(modb)
    ga_v[...] = modb_c[0:D]
    sb_v[...] = modb_c[D:2 * D]
    cb_v[...] = _b(1.0 + modb_c[2 * D:3 * D])
    gb_v[...] = modb_c[3 * D:4 * D]
    wr_v[...] = _cols(wr_ref[...].astype(F32).reshape(1, D))

    cp_wo.wait()
    lane = lax.broadcasted_iota(jnp.int32, (8, 128), 1)
    sub = lax.broadcasted_iota(jnp.int32, (8, 128), 0)
    keys = [jnp.zeros((8, 128), jnp.int32), jnp.zeros((8, 128), jnp.int32)]
    nl = R3 // 128
    for t in range(S // R3):
        cols = slice(t * R3, (t + 1) * R3)
        ocat = jnp.concatenate([o_v[hq, cols, :] for hq in range(HQ)], axis=1)
        att = _b(lax.dot_general(wo_v[...], ocat, NT, preferred_element_type=F32))
        x1 = _b(x_v[:, cols].astype(F32) + _b(_tile_lanes(ga_v, nl) * att))
        x_v[:, cols] = x1.astype(BF)
        h2 = _ln_mod_t(x1, _tile_lanes(cb_v, nl), _tile_lanes(sb_v, nl))
        out_v[:, cols] = (x1 + _b(_tile_lanes(gb_v, nl) * h2)).astype(BF)
        r = _b(jnp.sum(h2 * _tile_lanes(wr_v, nl), axis=0, keepdims=True))
        for i in range(nl):
            tt = t * nl + i
            rb = pltpu.bitcast(jnp.broadcast_to(r[:, i * 128:(i + 1) * 128], (8, 128)), jnp.int32)
            u = jnp.right_shift(rb, 16)
            u = jnp.where(u < 0, u ^ 0x7FFF, u) + 32768
            keys[tt // 8] = jnp.where(sub == tt % 8, u, keys[tt // 8])
    kf = []
    for b in range(2):
        tok = (sub + 8 * b) * 128 + lane
        kb = (keys[b] << 11) + (S - 1 - tok) + 0x00800000
        kf.append(pltpu.bitcast(kb, F32))

    lane_d = lax.broadcasted_iota(jnp.int32, (D // 2, 128), 1)
    xg = jnp.zeros((D // 2, 128), U32)
    r_sel = jnp.zeros((8, 128), F32)
    idxs = []
    for i in range(C):
        mx = jnp.max(jnp.maximum(kf[0], kf[1]), axis=1, keepdims=True)
        mx = jnp.max(mx, axis=0, keepdims=True)
        kf = [jnp.where(k == mx, 0.0, k) for k in kf]
        mi = pltpu.bitcast(jnp.broadcast_to(mx, (8, 128)), jnp.int32) - 0x00800000
        uu = jnp.right_shift(mi, 11) - 32768
        uu = jnp.where(uu < 0, uu ^ 0x7FFF, uu)
        r_sel = jnp.where(lane == i, pltpu.bitcast(uu << 16, F32), r_sel)
        idx = (S - 1) - (mi[0, 0] & (S - 1))
        idxs.append(idx)
        t0 = pl.multiple_of((idx >> 7) << 7, 128)
        tile = pltpu.bitcast(x_v[:, pl.ds(t0, 128)], U32)
        tile = pltpu.roll(tile, (i - (idx & 127)) & 127, 1)
        xg = jnp.where(lane_d == i, tile, xg)

    x1_sel = pltpu.bitcast(xg, BF).astype(F32)
    h_sel = _ln_mod_t(x1_sel, cb_v[...], sb_v[...])
    hb = h_sel.T[0:16].astype(BF)
    cp_wg.wait(); cp_wu.wait(); cp_wd.wait()
    gate = _b(jnp.dot(hb, wg_v[...], preferred_element_type=F32))
    up = _b(jnp.dot(hb, wu_v[...], preferred_element_type=F32))
    act = _b(_b(gate * _sigmoid_b(gate)) * up)
    y = _b(lax.dot_general(act.astype(BF), wd_v[...], NT, preferred_element_type=F32))
    yt = jnp.concatenate([y, jnp.zeros((128 - 16, D), F32)], axis=0).T
    yt = _b(yt * _sigmoid_b(r_sel[0:1]))
    new_c = (x1_sel + _b(gb_v[...] * _b(h_sel + yt))).astype(BF)
    new_p = pltpu.bitcast(new_c, U32)
    for i in range(C):
        idx = idxs[i]
        t0 = pl.multiple_of((idx >> 7) << 7, 128)
        tile = pltpu.bitcast(out_v[:, pl.ds(t0, 128)], U32)
        rolled = pltpu.roll(new_p, ((idx & 127) - i) & 127, 1)
        out_v[:, pl.ds(t0, 128)] = pltpu.bitcast(jnp.where(lane_d == (idx & 127), rolled, tile), BF)

    cp_out.start()
    cp_out.wait()


@jax.jit
def pallas_adaLN_cond__gqa_block_cached__moe_arch_mod__prompt_kernel(
    A_x: jax.Array,
    A_k_cache: jax.Array,
    A_v_cache: jax.Array,
    A_wq: jax.Array,
    A_wo: jax.Array,
    B_x: jax.Array,
    B_w_r: jax.Array,
    B_w_gate: jax.Array,
    B_w_up: jax.Array,
    B_w_down: jax.Array,
    c: jax.Array,
    w_mod: jax.Array,
):
    del B_x
    any_spec = pl.BlockSpec(memory_space=pl.ANY)
    vmem_spec = pl.BlockSpec(memory_space=pltpu.VMEM)
    n_sems = 1 + S // R1 + (HQ * DH) // NQ + 8
    col = pltpu.VMEM((D, 128), F32)
    out_t = pl.pallas_call(
        _kernel,
        out_shape=jax.ShapeDtypeStruct((1, D, S), BF),
        in_specs=[any_spec, any_spec, any_spec, any_spec, any_spec, vmem_spec,
                  any_spec, any_spec, any_spec, vmem_spec, any_spec],
        out_specs=any_spec,
        scratch_shapes=[
            pltpu.VMEM((D, S), BF),
            pltpu.VMEM((HKV, SK, DH), BF),
            pltpu.VMEM((HKV, SK, DH), BF),
            pltpu.VMEM((D, HQ * DH), BF),
            pltpu.VMEM((D, HQ * DH), BF),
            pltpu.VMEM((D, F), BF),
            pltpu.VMEM((D, F), BF),
            pltpu.VMEM((D, F), BF),
            pltpu.VMEM((D, 6 * D), BF),
            pltpu.VMEM((HQ, S, DH), BF),
            pltpu.VMEM((HQ, S, DH), BF),
            pltpu.VMEM((D, S), BF),
            col, col, col, col, col, col, col,
            pltpu.SemaphoreType.DMA((n_sems,)),
        ],
        compiler_params=pltpu.CompilerParams(vmem_limit_bytes=110 * 1024 * 1024),
        name="adaln_gqa_moe",
    )(jnp.swapaxes(A_x, 1, 2), A_k_cache, A_v_cache, A_wq, A_wo.T, B_w_r, B_w_gate, B_w_up, B_w_down.T, c, w_mod)
    return jnp.swapaxes(out_t, 1, 2)
```

```python
import numpy as np
import jax
import jax.numpy as jnp
from jax import lax
import jax.experimental.pallas as pl
import jax.experimental.pallas.tpu as pltpu

S = 2048
D = 576
HQ, HKV, DH = 32, 16, 128
SK = 2048
F = 4608
C = 8

BF = jnp.bfloat16
F32 = jnp.float32
U32 = jnp.uint32
NT = (((1,), (1,)), ((), ()))

LOG2E = 1.4426950408889634
QSCALE = (DH ** -0.5) * LOG2E
EPS_BF = 1.0013580322265625e-05

R1 = 256
RA = 128
CK = 512
R3 = 128
NQ = 512
XB = [0, R1, 2 * R1, 3 * R1, S]
WB = [0, 512, 1024, 2048, 3072, 4096]
PJ = 0
MODB1 = 0
UNROLLED1 = 5


def _b(x):
    return x.astype(BF).astype(F32)


def _vsum(x):
    return jnp.sum(x.reshape(x.shape[0] // 8, 8, x.shape[1]), axis=0)


def _sigmoid_b(x):
    return _b(1.0 / _b(1.0 + _b(jnp.exp(-x))))


def _cols(row):
    return jnp.broadcast_to(row, (128, row.shape[1])).T


def _lanes(v, n):
    return jnp.concatenate([v] * n, axis=1) if n > 1 else v


def _pad_rows(x, n):
    if x.shape[0] == n:
        return x
    return jnp.concatenate([x, jnp.zeros((n - x.shape[0], x.shape[1]), x.dtype)], axis=0)


def _slab(x):
    if x.dtype == BF:
        return x[x.shape[0] - 16:, 0:128]
    x = x[x.shape[0] - 8:, 0:128]
    return jnp.concatenate([x, x], axis=0).astype(BF)


def _fold(x):
    u = pltpu.bitcast(x, U32)
    acc = u[0:8]
    for i in range(1, u.shape[0] // 8):
        acc = acc | u[8 * i:8 * i + 8]
    return pltpu.bitcast(acc, BF)


def _join(a, b):
    return pltpu.bitcast(pltpu.bitcast(a, U32) | pltpu.bitcast(b, U32), BF)


def _pin(w, deps, never):
    if all(d is None for d in deps):
        return w
    tops = []
    for i, d in enumerate(deps):
        t = w[0:16, i * 128:(i + 1) * 128]
        tops.append(t if d is None else jnp.where(never, d, t))
    if w.shape[1] > 128 * len(deps):
        tops.append(w[0:16, 128 * len(deps):])
    top = tops[0] if len(tops) == 1 else jnp.concatenate(tops, axis=1)
    return jnp.concatenate([top, w[16:]], axis=0)


def _inv_std(sumsq):
    var = jnp.sum(sumsq, axis=0, keepdims=True) * (1.0 / D)
    return 1.0 / _b(jnp.sqrt(_b(_b(var) + EPS_BF)))


def _rows(bounds):
    return [slice(a, b) for a, b in zip(bounds[:-1], bounds[1:])]


class _Pieces:
    def __init__(self, gen=None):
        self.gen = iter(()) if gen is None else gen

    def step(self, k=1):
        dep = None
        for _ in range(k):
            d = next(self.gen, None)
            dep = d if d is not None else dep
        return dep

    def drain(self):
        for _ in self.gen:
            pass


def _kernel(x_hbm, k_hbm, v_hbm, wq_hbm, wo_hbm, wr_ref, wg_hbm, wu_hbm, wd_hbm, c_ref, wm_hbm, zero_ref,
            out_hbm,
            x_v, k_v, v_v, wq_v, wo_v, wg_v, wu_v, wd_v, wdn_v, wm_v, q_v, o_v, out_v, h2r_v, h_v,
            sa_v, ca_v, ga_v, sb_v, cb_v, gb_v, wr_v, gbr_v, key_v, acc_v, l_v, sems):
    never = zero_ref[0] != 0
    nx = S // R1
    nq = (HQ * DH) // NQ

    def colcopy(src, dst, lo, hi, sem):
        return pltpu.make_async_copy(src.at[:, pl.ds(lo, hi - lo)], dst.at[:, pl.ds(lo, hi - lo)], sems.at[sem])

    cp_wma = colcopy(wm_hbm, wm_v, 0, 2 * D, 0)
    cp_wmb = colcopy(wm_hbm, wm_v, 2 * D, 6 * D, 1)
    cp_x = [colcopy(x_hbm.at[0], x_v, XB[i], XB[i + 1], 2 + i) for i in range(len(XB) - 1)]
    cp_wq = [colcopy(wq_hbm, wq_v, WB[i], WB[i + 1], 6 + i) for i in range(len(WB) - 1)]
    cp_k = pltpu.make_async_copy(k_hbm.at[0], k_v, sems.at[11])
    cp_v = pltpu.make_async_copy(v_hbm.at[0], v_v, sems.at[12])
    cp_wo = pltpu.make_async_copy(wo_hbm, wo_v, sems.at[13])
    cp_wg = pltpu.make_async_copy(wg_hbm, wg_v, sems.at[14])
    cp_wu = pltpu.make_async_copy(wu_hbm, wu_v, sems.at[15])
    cp_wd = pltpu.make_async_copy(wd_hbm, wd_v, sems.at[16])
    cp_out = pltpu.make_async_copy(out_v, out_hbm.at[0], sems.at[17])
    PATCH_SEM = 18

    cp_wma.start()
    cp_x[0].start()
    cp_wq[0].start()

    c = c_ref[...].astype(F32)
    sc = _b(c * _sigmoid_b(c)).astype(BF)
    sc8 = jnp.broadcast_to(sc, (8, D))
    cp_wma.wait()
    moda = _b(jnp.dot(sc8, wm_v[:, 0:2 * D], preferred_element_type=F32))[0:1]
    moda_c = _cols(moda)
    sa_v[...] = moda_c[0:D]
    ca_v[...] = _b(1.0 + moda_c[D:2 * D])

    KP = _rows([0, 128, 256, 384, 512, D])
    nl1 = R1 // 128

    def ln1(t):
        cols = pl.ds(pl.multiple_of(jnp.minimum(t, nx - 1) * R1, R1), R1)
        xs = [x_v[r, cols].astype(F32) for r in KP]
        tot = _vsum(xs[0])
        for xp in xs[1:]:
            tot = tot + _vsum(xp)
        yield _slab(tot)
        mean = jnp.sum(tot, axis=0, keepdims=True) * (1.0 / D)
        tot = None
        for xp in xs:
            xc = xp - mean
            tot = _vsum(xc * xc) if tot is None else tot + _vsum(xc * xc)
        yield _slab(tot)
        inv = _inv_std(tot)
        mean_b = _b(mean)
        for i, (r, xp) in enumerate(zip(KP, xs)):
            hn = _b(_b(xp - mean_b) * inv)
            hv = _b(hn * _lanes(ca_v[r, :], nl1)) + _lanes(sa_v[r, :], nl1)
            h_v[t % 2, :, i * 128:(i + 1) * 128] = _pad_rows(hv.astype(BF), 128).T
            yield _fold(h_v[t % 2, :, i * 128:(i + 1) * 128])

    def mod_b():
        for i, (dst, plus1) in enumerate([(ga_v, False), (sb_v, False), (cb_v, True), (gb_v, False)]):
            if i % 2 == 0:
                modb = _b(jnp.dot(sc8, wm_v[:, (2 + i) * D:(4 + i) * D], preferred_element_type=F32))
                modb_c = _cols(modb[0:1])
            val = modb_c[(i % 2) * D:(i % 2 + 1) * D]
            val = _b(1.0 + val) if plus1 else val
            dst[...] = val
            if i == 3:
                gbr_v[...] = modb[:, D:2 * D]
            yield _slab(val)
        val = _cols(wr_ref[...].astype(F32).reshape(1, D))
        wr_v[...] = val
        yield _slab(val)

    first = {
        0: ([cp_wq[0]], [cp_wq[2]]),
        1: ([cp_wq[1]], [cp_x[1]]),
        2: ([cp_wq[2]], [cp_wq[3], cp_x[2]]),
        4: ([cp_wq[3], cp_x[1]], [cp_wq[4]]),
        6: ([cp_wq[4], cp_x[2]], [cp_x[3]]),
    }
    def q_tile(t, pcs, first_tile=False):
        h = h_v[t % 2, :, 0:D]
        rows = pl.ds(pl.multiple_of(t * R1, R1), R1)
        dep = None
        for n in range(nq):
            if first_tile and n in first:
                for cp in first[n][0]:
                    cp.wait()
                for cp in first[n][1]:
                    cp.start()
            w = _pin(wq_v[:, n * NQ:(n + 1) * NQ], [dep], never)
            qn = jnp.dot(h, w, preferred_element_type=F32) * QSCALE
            for i in range(NQ // DH):
                q_v[n * (NQ // DH) + i, rows, :] = qn[:, i * DH:(i + 1) * DH].astype(BF)
            if not first_tile:
                dep = pcs.step()
            elif n >= 4:
                dep = pcs.step(2)
        pcs.drain()

    cp_x[0].wait()
    cp_wq[1].start()
    _Pieces(ln1(0)).drain()
    for t in range(UNROLLED1):
        if t == 2:
            cp_x[3].wait()
            cp_k.start(); cp_v.start(); cp_wmb.start()
        q_tile(t, _Pieces(ln1(t + 1)), first_tile=(t == 0))

    def q_body(t, carry):
        q_tile(t, _Pieces(ln1(t + 1)))
        return carry

    lax.fori_loop(UNROLLED1, nx, q_body, 0)

    nck = SK // CK
    rep = HQ // HKV

    def finalize(acc, l, hq, t0):
        lsum = jnp.sum(l, axis=1, keepdims=True)
        rl = pl.reciprocal(lsum, approx=True)
        rl = rl * (2.0 - lsum * rl)
        o_v[hq, pl.ds(t0, RA), :] = (acc * rl).astype(BF)

    def attn_body(g, carry):
        tiles = [(hh, t) for hh in range(rep) for t in range(S // RA)]
        steps = [(ti, j) for ti in range(len(tiles)) for j in range(nck)]

        def qk(ti, j, dep=None):
            hh, t = tiles[ti]
            q = q_v[g * rep + hh, t * RA:(t + 1) * RA, :]
            return lax.dot_general(q, _pin(k_v[g, j * CK:(j + 1) * CK, :], [dep], never), NT,
                                   preferred_element_type=F32)

        s = qk(0, 0)
        prev_head = jnp.where(g == 0, HQ, g * rep - 1)
        finalize(acc_v[...], l_v[...], prev_head, S - RA)
        dep = _fold(o_v[prev_head, S - RA:S, :])
        m = l = acc = None
        for n, (ti, j) in enumerate(steps):
            s_next = None
            if n + 1 < len(steps):
                s_next = qk(*steps[n + 1], dep=dep if (PJ > 0 and j == PJ) else None)
            cm = s[:, 0:128]
            for i in range(1, CK // 128):
                cm = jnp.maximum(cm, s[:, i * 128:(i + 1) * 128])
            cm = jnp.max(cm, axis=1, keepdims=True)
            if m is None:
                m_new, alpha = cm, None
            else:
                m_new = jnp.maximum(m, cm)
                alpha = jnp.exp2(m - m_new)
            p = jnp.exp2(s - m_new)
            ls = p[:, 0:128]
            for i in range(1, CK // 128):
                ls = ls + p[:, i * 128:(i + 1) * 128]
            l = ls if l is None else alpha * l + ls
            o = jnp.dot(p.astype(BF), v_v[g, j * CK:(j + 1) * CK, :], preferred_element_type=F32)
            acc = o if acc is None else alpha * acc + o
            m = m_new
            if j == nck - 1:
                hh, t = tiles[ti]
                if ti + 1 < len(tiles):
                    finalize(acc, l, g * rep + hh, t * RA)
                    dep = _fold(o_v[g * rep + hh, t * RA:(t + 1) * RA, :])
                else:
                    acc_v[...] = acc
                    l_v[...] = l
                m = l = acc = None
            s = s_next
        return carry

    acc_v[...] = jnp.zeros((RA, DH), F32)
    l_v[...] = jnp.ones((RA, 128), F32)
    cp_k.wait()
    cp_v.wait()
    cp_wo.start(); cp_wg.start(); cp_wu.start(); cp_wd.start()
    lax.fori_loop(0, HKV, attn_body, 0)
    finalize(acc_v[...], l_v[...], HQ - 1, S - RA)

    lane = lax.broadcasted_iota(jnp.int32, (8, 128), 1)
    KC = 512
    nkc = HQ * DH // KC
    H2 = _rows([0, 288, D])

    def out_proj_chunk(t, kc, deps):
        cols = slice(t * R3, (t + 1) * R3)
        hpc = KC // DH
        ocat = jnp.concatenate([o_v[kc * hpc + i, cols, :] for i in range(hpc)], axis=1)
        return lax.dot_general(wo_v[:, kc * KC:(kc + 1) * KC], _pin(ocat, deps, never), NT,
                               preferred_element_type=F32)

    def epilogue(t, att):
        cols = slice(t * R3, (t + 1) * R3)
        tot = None
        for r in H2:
            x1 = _b(x_v[r, cols].astype(F32) + _b(ga_v[r, :] * _b(att[r])))
            x_v[r, cols] = x1.astype(BF)
            tot = _vsum(x1) if tot is None else tot + _vsum(x1)
            yield _slab(tot)
        mean = jnp.sum(tot, axis=0, keepdims=True) * (1.0 / D)
        xs = [x_v[r, cols].astype(F32) for r in KP]
        tot = None
        for xp in xs:
            xc = xp - mean
            tot = _vsum(xc * xc) if tot is None else tot + _vsum(xc * xc)
        yield _slab(tot)
        inv = _inv_std(tot)
        mean_b = _b(mean)
        rs = None
        for i, (r, xp) in enumerate(zip(KP, xs)):
            hn = _b(_b(xp - mean_b) * inv)
            h2b = (_b(hn * cb_v[r, :]) + sb_v[r, :]).astype(BF)
            h2 = h2b.astype(F32)
            out_v[r, cols] = (xp + _b(gb_v[r, :] * h2)).astype(BF)
            rp = _vsum(h2 * wr_v[r, :])
            rs = rp if rs is None else rs + rp
            h2r_v[cols, i * 128:(i + 1) * 128] = _pad_rows(h2b, 128).T
            dep = _join(_slab(rs), _fold(h2r_v[cols, i * 128:(i + 1) * 128]))
            if i + 1 < len(KP):
                yield dep
        r = _b(jnp.sum(rs, axis=0, keepdims=True))
        rb = pltpu.bitcast(jnp.broadcast_to(r, (8, 128)), jnp.int32)
        u = jnp.right_shift(rb, 16)
        u = jnp.where(u < 0, u ^ 0x7FFF, u) + 32768
        tok = t * 128 + lane
        kb = (u << 11) + (S - 1 - tok) + 0x00800000
        key_v[t:t + 1, :] = pltpu.bitcast(kb, F32)[0:1]
        yield dep

    def wd_transpose():
        for j in range(F // 128):
            blk = _pad_rows(wd_v[:, j * 128:(j + 1) * 128], 640).T[:, 0:D]
            wdn_v[j * 128:(j + 1) * 128, :] = blk
            back = wdn_v[j * 128:(j + 1) * 128, :]
            dep = _fold(back[:, 0:128])
            for i in range(1, 4):
                dep = _join(dep, _fold(back[:, i * 128:(i + 1) * 128]))
            last = back[112:128, 448:D]
            yield _join(dep, last)

    cp_wo.wait()
    cp_wd.wait()
    if not MODB1:
        cp_wmb.wait()
    pcs = _Pieces() if MODB1 else _Pieces(mod_b())
    wds = _Pieces(wd_transpose())
    for t in range(S // R3):
        att = None
        dep = dep2 = None
        for kc in range(nkc):
            part = out_proj_chunk(t, kc, [dep, dep2])
            att = part if att is None else att + part
            dep = pcs.step()
            dep2 = wds.step() if (t >= 1 and kc % 3 == 0) else None
        pcs.drain()
        pcs = _Pieces(epilogue(t, att))
    wds.drain()
    pcs.drain()
    cp_out.start()

    lane_d = lax.broadcasted_iota(jnp.int32, (D // 2, 128), 1)
    sub = lax.broadcasted_iota(jnp.int32, (8, 128), 0)
    sub16 = lax.broadcasted_iota(jnp.int32, (16, D), 0)
    sub8 = lax.broadcasted_iota(jnp.int32, (8, D), 0)
    kf = [key_v[0:8, :], key_v[8:16, :]]
    xg = jnp.zeros((D // 2, 128), U32)
    h_sel = jnp.zeros((8, D), F32)
    r_sel = jnp.zeros((8, 128), F32)
    idxs = []
    for i in range(C):
        mx = jnp.max(jnp.maximum(kf[0], kf[1]), axis=1, keepdims=True)
        mx = jnp.max(mx, axis=0, keepdims=True)
        kf = [jnp.where(k == mx, 0.0, k) for k in kf]
        mi = pltpu.bitcast(jnp.broadcast_to(mx, (8, 128)), jnp.int32) - 0x00800000
        uu = jnp.right_shift(mi, 11) - 32768
        uu = jnp.where(uu < 0, uu ^ 0x7FFF, uu)
        r_sel = jnp.where(sub == i, pltpu.bitcast(uu << 16, F32), r_sel)
        idx = (S - 1) - (mi[0, 0] & (S - 1))
        idxs.append(idx)
        b16 = pl.multiple_of((idx >> 4) << 4, 16)
        tile = h2r_v[pl.ds(b16, 16), 0:D].astype(F32)
        row = jnp.sum(jnp.where(sub16 == (idx & 15), tile, 0.0), axis=0, keepdims=True)
        h_sel = jnp.where(sub8 == i, row, h_sel)
        t0 = pl.multiple_of((idx >> 7) << 7, 128)
        tile = pltpu.bitcast(x_v[:, pl.ds(t0, 128)], U32)
        tile = pltpu.roll(tile, (i - (idx & 127)) & 127, 1)
        xg = jnp.where(lane_d == i, tile, xg)

    hb = _pad_rows(h_sel, 16).astype(BF)
    cp_wg.wait(); cp_wu.wait()
    gate = _b(jnp.dot(hb, wg_v[...], preferred_element_type=F32)[0:8])
    up = _b(jnp.dot(hb, wu_v[...], preferred_element_type=F32)[0:8])
    act = _b(_b(gate * _sigmoid_b(gate)) * up)
    y = _b(jnp.dot(_pad_rows(act, 16).astype(BF), wdn_v[...], preferred_element_type=F32)[0:8])
    x1_sel = _pad_rows(pltpu.bitcast(xg, BF), 640).T[0:8, 0:D].astype(F32)
    y = _b(y * _lanes(_sigmoid_b(r_sel), 5)[:, 0:D])
    new = (x1_sel + _b(gbr_v[...] * _b(h_sel + y))).astype(BF)
    new_c = _pad_rows(new, 128)
    new_c = jnp.concatenate([new_c, jnp.zeros((128, 640 - D), BF)], axis=1).T[0:D]
    new_p = pltpu.bitcast(new_c, U32)
    cp_out.wait()
    for i in range(C):
        idx = idxs[i]
        t0 = pl.multiple_of((idx >> 7) << 7, 128)
        tile = pltpu.bitcast(out_v[:, pl.ds(t0, 128)], U32)
        rolled = pltpu.roll(new_p, ((idx & 127) - i) & 127, 1)
        out_v[:, pl.ds(t0, 128)] = pltpu.bitcast(jnp.where(lane_d == (idx & 127), rolled, tile), BF)

    patches = []
    for i in range(C):
        ti = idxs[i] >> 7
        fresh = ti >= 0
        for j in range(i):
            fresh = jnp.logical_and(fresh, ti != (idxs[j] >> 7))
        t0 = pl.multiple_of(ti << 7, 128)
        cp = pltpu.make_async_copy(out_v.at[:, pl.ds(t0, 128)], out_hbm.at[0, :, pl.ds(t0, 128)],
                                   sems.at[PATCH_SEM + i])
        patches.append((fresh, cp))
        pl.when(fresh)(cp.start)
    for fresh, cp in patches:
        pl.when(fresh)(cp.wait)


@jax.jit
def pallas_adaLN_cond__gqa_block_cached__moe_arch_mod__prompt_kernel(
    A_x, A_k_cache, A_v_cache, A_wq, A_wo, B_x, B_w_r, B_w_gate, B_w_up, B_w_down, c, w_mod,
):
    del B_x
    any_spec = pl.BlockSpec(memory_space=pl.ANY)
    vmem_spec = pl.BlockSpec(memory_space=pltpu.VMEM)
    col = pltpu.VMEM((D, 128), F32)
    out_t = pl.pallas_call(
        _kernel,
        out_shape=jax.ShapeDtypeStruct((1, D, S), BF),
        in_specs=[any_spec, any_spec, any_spec, any_spec, any_spec, vmem_spec,
                  any_spec, any_spec, any_spec, vmem_spec, any_spec,
                  pl.BlockSpec(memory_space=pltpu.SMEM)],
        out_specs=any_spec,
        scratch_shapes=[
            pltpu.VMEM((D, S), BF),
            pltpu.VMEM((HKV, SK, DH), BF),
            pltpu.VMEM((HKV, SK, DH), BF),
            pltpu.VMEM((D, HQ * DH), BF),
            pltpu.VMEM((D, HQ * DH), BF),
            pltpu.VMEM((D, F), BF),
            pltpu.VMEM((D, F), BF),
            pltpu.VMEM((D, F), BF),
            pltpu.VMEM((F, D), BF),
            pltpu.VMEM((D, 6 * D), BF),
            pltpu.VMEM((HQ, S, DH), BF),
            pltpu.VMEM((HQ + 1, S, DH), BF),
            pltpu.VMEM((D, S), BF),
            pltpu.VMEM((S, 640), BF),
            pltpu.VMEM((2, R1, 640), BF),
            col, col, col, col, col, col, col,
            pltpu.VMEM((8, D), F32),
            pltpu.VMEM((16, 128), F32),
            pltpu.VMEM((RA, DH), F32),
            pltpu.VMEM((RA, 128), F32),
            pltpu.SemaphoreType.DMA((18 + C,)),
        ],
        compiler_params=pltpu.CompilerParams(vmem_limit_bytes=120 * 1024 * 1024),
        name="adaln_gqa_moe",
    )(jnp.swapaxes(A_x, 1, 2), A_k_cache, A_v_cache, A_wq, A_wo.T, B_w_r, B_w_gate, B_w_up, B_w_down.T, c, w_mod,
      np.zeros((1,), np.int32))
    return jnp.swapaxes(out_t, 1, 2)
```

```python
import numpy as np
import jax
import jax.numpy as jnp
from jax import lax
import jax.experimental.pallas as pl
import jax.experimental.pallas.tpu as pltpu

S = 2048
D = 576
HQ, HKV, DH = 32, 16, 128
SK = 2048
F = 4608
C = 8

BF = jnp.bfloat16
F32 = jnp.float32
U32 = jnp.uint32
NT = (((1,), (1,)), ((), ()))

LOG2E = 1.4426950408889634
QSCALE = (DH ** -0.5) * LOG2E
EPS_BF = 1.0013580322265625e-05

R1 = 256
RA = 128
CK = 512
R3 = 128
NQ = 512
PLANS = {
    0: ([0, 256, 512, 1024, S], [0, 512, 1536, 2560, 4096], "wm x0 w0 x1 w1 w2 w3 x2 x3", "", "",
        {0: ("w0 x1", ""), 2: ("w1", ""), 6: ("w2", ""), 10: ("w3 x2", "")}),
    1: ([0, 256, 512, 1024, S], [0, 512, 1024, 2048, 4096], "wm x0 w0 x1 w1 w2 w3 x2 x3", "", "",
        {0: ("w0 x1", ""), 2: ("w1", ""), 4: ("w2", ""), 8: ("w3 x2", "")}),
    2: ([0, 256, 512, 1024, S], [0, 512, 1024, 2560, 4096], "wm x0 w0 x1 w1 w2 x2 w3 x3", "", "",
        {0: ("w0 x1", ""), 2: ("w1", ""), 4: ("w2 x2", ""), 10: ("w3", "")}),
    5: ([0, 512, 768, S], [0, 512, 1536, 2560, 4096], "wm x0 w0", "w1", "",
        {0: ("w0", "w2"), 2: ("w1", "w3"), 6: ("w2", "x1"), 10: ("w3 x1", "x2")}),
}
PLAN = 5
XB, WB, ST0, ST_WM, ST_X0, FIRST = PLANS[PLAN]
STAGED = PLAN >= 5
LN2_AT = max(i for i, (w, _) in FIRST.items() if ('x1' if STAGED else 'x2') in w.split())
PJ = 2
MODB1 = 0
LAG = 0
WDP = 3
WDO = 0
VARY = (1,)
S3Y = 3
NLATE = 1
RELOAD = 1
SUBV = 0
PINX = 1
UNROLLED1 = 5


def _b(x):
    return x.astype(BF).astype(F32)


def _vsum(x):
    return jnp.sum(x.reshape(x.shape[0] // 8, 8, x.shape[1]), axis=0)


def _sub_row(x, row):
    if not SUBV:
        return x - row
    n = x.shape[0] // 8
    r8 = jnp.broadcast_to(row, (8, 128))
    return (x.reshape(n, 8, 128) - r8[None]).reshape(8 * n, 128)


def _sigmoid_b(x):
    return _b(1.0 / _b(1.0 + _b(jnp.exp(-x))))


def _cols(row):
    return jnp.broadcast_to(row, (128, row.shape[1])).T


def _lanes(v, n):
    return jnp.concatenate([v] * n, axis=1) if n > 1 else v


def _pad_rows(x, n):
    if x.shape[0] == n:
        return x
    return jnp.concatenate([x, jnp.zeros((n - x.shape[0], x.shape[1]), x.dtype)], axis=0)


def _slab(x):
    if x.dtype == BF:
        return x[x.shape[0] - 16:, 0:128]
    x = x[x.shape[0] - 8:, 0:128]
    return jnp.concatenate([x, x], axis=0).astype(BF)


def _fold(x):
    u = pltpu.bitcast(x, U32)
    acc = u[0:8]
    for i in range(1, u.shape[0] // 8):
        acc = acc | u[8 * i:8 * i + 8]
    return pltpu.bitcast(acc, BF)


def _join(a, b):
    return pltpu.bitcast(pltpu.bitcast(a, U32) | pltpu.bitcast(b, U32), BF)


def _late(d):
    u = pltpu.bitcast(d, U32)
    for _ in range(NLATE):
        u = pltpu.roll(u, 1, 1)
    return pltpu.bitcast(u, BF)


def _pin(w, deps, never, late=True):
    if all(d is None for d in deps):
        return w
    deps = [None if d is None else (_late(d) if late else d) for d in deps]
    tops = []
    for i, d in enumerate(deps):
        t = w[0:16, i * 128:(i + 1) * 128]
        tops.append(t if d is None else jnp.where(never, d, t))
    if w.shape[1] > 128 * len(deps):
        tops.append(w[0:16, 128 * len(deps):])
    top = tops[0] if len(tops) == 1 else jnp.concatenate(tops, axis=1)
    return jnp.concatenate([top, w[16:]], axis=0)


def _inv_std(sumsq):
    var = jnp.sum(sumsq, axis=0, keepdims=True) * (1.0 / D)
    return 1.0 / _b(jnp.sqrt(_b(_b(var) + EPS_BF)))


def _rows(bounds):
    return [slice(a, b) for a, b in zip(bounds[:-1], bounds[1:])]


class _Pieces:
    def __init__(self, gen=None):
        self.gen = iter(()) if gen is None else gen

    def step(self, k=1):
        dep = None
        for _ in range(k):
            d = next(self.gen, None)
            dep = d if d is not None else dep
        return dep

    def drain(self):
        for _ in self.gen:
            pass


def _kernel(x_hbm, k_hbm, v_hbm, wq_hbm, wo_hbm, wr_hbm, wg_hbm, wu_hbm, wd_hbm, c_hbm, wm_hbm, zero_ref,
            out_hbm,
            x_v, k_v, v_v, wq_v, wo_v, wg_v, wu_v, wd_v, wdn_v, wm_v, q_v, o_v, out_v, h2r_v, h_v,
            c_ref, wr_ref, sa_v, ca_v, ga_v, sb_v, cb_v, gb_v, wr_v, gbr_v, key_v, cand_v, acc_v, l_v, sems):
    never = zero_ref[0] != 0
    nx = S // R1
    nq = (HQ * DH) // NQ

    def colcopy(src, dst, lo, hi, sem):
        return pltpu.make_async_copy(src.at[:, pl.ds(lo, hi - lo)], dst.at[:, pl.ds(lo, hi - lo)], sems.at[sem])

    cp_wma = colcopy(wm_hbm, wm_v, 0, 2 * D, 0)
    cp_wmb = colcopy(wm_hbm, wm_v, 2 * D, 6 * D, 1)
    cp_x = [colcopy(x_hbm.at[0], x_v, XB[i], XB[i + 1], 2 + i) for i in range(len(XB) - 1)]
    cp_wq = [colcopy(wq_hbm, wq_v, WB[i], WB[i + 1], 6 + i) for i in range(len(WB) - 1)]
    WS = 1
    cp_k = pltpu.make_async_copy(k_hbm.at[0], k_v, sems.at[12])
    cp_v = pltpu.make_async_copy(v_hbm.at[0], v_v, sems.at[13])
    cp_wo = pltpu.make_async_copy(wo_hbm, wo_v, sems.at[14])
    cp_wg = pltpu.make_async_copy(wg_hbm, wg_v, sems.at[15])
    cp_wu = pltpu.make_async_copy(wu_hbm, wu_v, sems.at[16])
    cp_wd = pltpu.make_async_copy(wd_hbm, wd_v, sems.at[17])
    cp_out = pltpu.make_async_copy(out_v, out_hbm.at[0], sems.at[18])
    PATCH_SEM = 21

    named = {"wm": cp_wma, **{f"x{i}": cp for i, cp in enumerate(cp_x)}, **{f"w{i}": cp for i, cp in enumerate(cp_wq)}}
    waited = set()

    def start(names):
        for n in names.split():
            named[n].start()

    def wait(names):
        for n in names.split():
            if n not in waited:
                named[n].wait()
                waited.add(n)

    cp_c = pltpu.make_async_copy(c_hbm, c_ref, sems.at[19])
    cp_wr = pltpu.make_async_copy(wr_hbm, wr_ref, sems.at[20])
    cp_c.start()
    start(ST0)
    cp_wr.start()
    if not STAGED:
        cp_k.start(); cp_v.start(); cp_wmb.start()
        cp_wo.start(); cp_wd.start(); cp_wg.start(); cp_wu.start()

    cp_c.wait()
    c = c_ref[...].astype(F32)
    sc = _b(c * _sigmoid_b(c)).astype(BF)
    sc8 = jnp.broadcast_to(sc, (8, D))
    wait("wm")
    start(ST_WM)
    moda = _b(jnp.dot(sc8, wm_v[:, 0:2 * D], preferred_element_type=F32))[0:1]
    moda_c = _cols(moda)
    sa_v[...] = moda_c[0:D]
    ca_v[...] = _b(1.0 + moda_c[D:2 * D])

    KP = _rows([0, 128, 256, 384, 512, D])
    nl1 = R1 // 128

    def ln1(t):
        cols = pl.ds(pl.multiple_of(jnp.minimum(t, nx - 1) * R1, R1), R1)
        xs = [x_v[r, cols].astype(F32) for r in KP]
        tot = _vsum(xs[0])
        for xp in xs[1:]:
            tot = tot + _vsum(xp)
        yield _slab(tot)
        mean = jnp.sum(tot, axis=0, keepdims=True) * (1.0 / D)
        tot = None
        for xp in xs:
            xc = xp - mean
            tot = _vsum(xc * xc) if tot is None else tot + _vsum(xc * xc)
        yield _slab(tot)
        inv = _inv_std(tot)
        mean_b = _b(mean)
        for i, (r, xp) in enumerate(zip(KP, xs)):
            hn = _b(_b(xp - mean_b) * inv)
            hv = _b(hn * _lanes(ca_v[r, :], nl1)) + _lanes(sa_v[r, :], nl1)
            h_v[t % 2, :, i * 128:(i + 1) * 128] = _pad_rows(hv.astype(BF), 128).T
            yield _fold(h_v[t % 2, :, i * 128:(i + 1) * 128])

    def mod_b():
        for i, (dst, plus1) in enumerate([(ga_v, False), (sb_v, False), (cb_v, True), (gb_v, False)]):
            if i % 2 == 0:
                modb = _b(jnp.dot(sc8, wm_v[:, (2 + i) * D:(4 + i) * D], preferred_element_type=F32))
                modb_c = _cols(modb[0:1])
            val = modb_c[(i % 2) * D:(i % 2 + 1) * D]
            val = _b(1.0 + val) if plus1 else val
            dst[...] = val
            if i == 3:
                gbr_v[...] = modb[:, D:2 * D]
            yield _slab(val)
        val = _cols(wr_ref[...].astype(F32).reshape(1, D))
        wr_v[...] = val
        yield _slab(val)

    def q_chunk(t, h, n, dep):
        rows = pl.ds(pl.multiple_of(t * R1, R1), R1)
        w = _pin(wq_v[:, n * NQ:(n + 1) * NQ], [dep], never)
        qn = jnp.dot(h, w, preferred_element_type=F32) * QSCALE
        for i in range(NQ // DH):
            q_v[n * (NQ // DH) + i, rows, :] = qn[:, i * DH:(i + 1) * DH].astype(BF)

    def q_tile(t, pcs):
        h = h_v[t % 2, :, 0:D]
        dep = None
        for n in range(nq):
            q_chunk(t, h, n, dep)
            dep = pcs.step()
        pcs.drain()

    wait("x0")
    start(ST_X0)
    _Pieces(ln1(0)).drain()
    h0 = h_v[0, :, 0:D]
    for i in range(2 * nq):
        t, n = i % 2, i // 2
        if i in FIRST:
            wait(FIRST[i][0])
            start(FIRST[i][1])
        if i == 0:
            dep = None
            pcs = _Pieces(ln1(1))
        elif i == 1:
            dep = pcs.step(7)
            h1 = h_v[1, :, 0:D]
        elif i == LN2_AT:
            dep = None
            pcs = _Pieces(ln1(2))
        elif i > LN2_AT:
            dep = pcs.step(1 if i < 2 * nq - 1 else 7)
        else:
            dep = None
        q_chunk(t, h0 if t == 0 else h1, n, dep)
    for t in range(2, UNROLLED1):
        if t == (2 if STAGED else 3):
            wait(" ".join(f"x{i}" for i in range(len(XB) - 1)))
            if STAGED:
                cp_k.start(); cp_v.start(); cp_wmb.start()
        q_tile(t, _Pieces(ln1(t + 1)))

    def q_body(t, carry):
        q_tile(t, _Pieces(ln1(t + 1)))
        return carry

    if UNROLLED1 < nx:
        lax.fori_loop(UNROLLED1, nx, q_body, 0)

    nck = SK // CK
    rep = HQ // HKV

    def finalize(acc, l, hq, t0):
        lsum = jnp.sum(l, axis=1, keepdims=True)
        rl = pl.reciprocal(lsum, approx=True)
        rl = rl * (2.0 - lsum * rl)
        ob = (acc * rl).astype(BF)
        o_v[hq, pl.ds(t0, RA), :] = ob
        return ob

    def attn_body(g, carry):
        tiles = [(hh, t) for hh in range(rep) for t in range(S // RA)]
        steps = [(ti, j) for ti in range(len(tiles)) for j in range(nck)]

        def qk(ti, j, dep=None):
            hh, t = tiles[ti]
            q = q_v[g * rep + hh, t * RA:(t + 1) * RA, :]
            return lax.dot_general(q, _pin(k_v[g, j * CK:(j + 1) * CK, :], [dep], never), NT,
                                   preferred_element_type=F32)

        s = qk(0, 0)
        prev_head = jnp.where(g == 0, HQ, g * rep - 1)
        dep = _fold(finalize(acc_v[...], l_v[...], prev_head, S - RA))
        m = l = acc = None
        for n, (ti, j) in enumerate(steps):
            s_next = None
            if n + 1 < len(steps):
                s_next = qk(*steps[n + 1], dep=dep if (PJ > 0 and j == PJ) else None)
            cm = s[:, 0:128]
            for i in range(1, CK // 128):
                cm = jnp.maximum(cm, s[:, i * 128:(i + 1) * 128])
            cm = jnp.max(cm, axis=1, keepdims=True)
            if m is None:
                m_new, alpha = cm, None
            else:
                m_new = jnp.maximum(m, cm)
                alpha = jnp.exp2(m - m_new)
            p = jnp.exp2(s - m_new)
            ls = p[:, 0:128]
            for i in range(1, CK // 128):
                ls = ls + p[:, i * 128:(i + 1) * 128]
            l = ls if l is None else alpha * l + ls
            o = jnp.dot(p.astype(BF), v_v[g, j * CK:(j + 1) * CK, :], preferred_element_type=F32)
            acc = o if acc is None else alpha * acc + o
            m = m_new
            if j == nck - 1:
                hh, t = tiles[ti]
                if ti + 1 < len(tiles):
                    dep = _fold(finalize(acc, l, g * rep + hh, t * RA))
                else:
                    acc_v[...] = acc
                    l_v[...] = l
                m = l = acc = None
            s = s_next
        return carry

    acc_v[...] = jnp.zeros((RA, DH), F32)
    l_v[...] = jnp.ones((RA, 128), F32)
    cp_k.wait()
    cp_v.wait()
    if STAGED:
        cp_wo.start(); cp_wd.start(); cp_wg.start(); cp_wu.start()
    lax.fori_loop(0, HKV, attn_body, 0)
    finalize(acc_v[...], l_v[...], HQ - 1, S - RA)

    lane = lax.broadcasted_iota(jnp.int32, (8, 128), 1)
    KC = 512
    nkc = HQ * DH // KC
    H2 = _rows([0, 288, D])

    def out_proj_chunk(t, kc, deps):
        cols = slice(t * R3, (t + 1) * R3)
        hpc = KC // DH
        ocat = jnp.concatenate([o_v[kc * hpc + i, cols, :] for i in range(hpc)], axis=1)
        return lax.dot_general(wo_v[:, kc * KC:(kc + 1) * KC], _pin(ocat, deps, never), NT,
                               preferred_element_type=F32)

    def epilogue(t, att):
        cols = slice(t * R3, (t + 1) * R3)
        tot = None
        for r in H2:
            x1 = _b(x_v[r, cols].astype(F32) + _b(ga_v[r, :] * _b(att[r])))
            x_v[r, cols] = x1.astype(BF)
            tot = _vsum(x1) if tot is None else tot + _vsum(x1)
            yield _slab(tot)
        mean = jnp.sum(tot, axis=0, keepdims=True) * (1.0 / D)
        tot = None
        xs_keep = []
        for i, r in enumerate(KP):
            xs_keep.append(x_v[r, cols])
            xc = _sub_row(xs_keep[i].astype(F32), mean)
            tot = _vsum(xc * xc) if tot is None else tot + _vsum(xc * xc)
            if i in VARY:
                yield _slab(tot)
        yield _slab(tot)
        inv = _inv_std(tot)
        mean_b = _b(mean)
        rs = None
        for i, r in enumerate(KP):
            xp = (x_v[r, cols] if RELOAD else xs_keep[i]).astype(F32)
            hn = _b(_b(xp - mean_b) * inv)
            h2b = (_b(hn * cb_v[r, :]) + sb_v[r, :]).astype(BF)
            h2 = h2b.astype(F32)
            out_v[r, cols] = (xp + _b(gb_v[r, :] * h2)).astype(BF)
            rp = _vsum(h2 * wr_v[r, :])
            rs = rp if rs is None else rs + rp
            h2r_v[cols, i * 128:(i + 1) * 128] = _pad_rows(h2b, 128).T
            d = _join(_slab(rs), _fold(h2r_v[cols, i * 128:(i + 1) * 128]))
            dep = d if i != len(KP) - 1 else _join(dep, d)
            if i < S3Y:
                yield dep
        r = _b(jnp.sum(rs, axis=0, keepdims=True))
        rb = pltpu.bitcast(jnp.broadcast_to(r, (8, 128)), jnp.int32)
        u = jnp.right_shift(rb, 16)
        u = jnp.where(u < 0, u ^ 0x7FFF, u) + 32768
        tok = t * 128 + lane
        kb = (u << 11) + (S - 1 - tok) + 0x00800000
        key_v[t:t + 1, :] = pltpu.bitcast(kb, F32)[0:1]
        yield dep

    def wd_transpose():
        for j in range(F // 128):
            blk = _pad_rows(wd_v[:, j * 128:(j + 1) * 128], 640).T[:, 0:D]
            wdn_v[j * 128:(j + 1) * 128, :] = blk
            back = wdn_v[j * 128:(j + 1) * 128, :]
            dep = _fold(back[:, 0:128])
            for i in range(1, 4):
                dep = _join(dep, _fold(back[:, i * 128:(i + 1) * 128]))
            last = back[112:128, 448:D]
            yield _join(dep, last)

    NLATEKEYS = 2

    def preselect():
        nt = S // R3 - NLATEKEYS
        sub = lax.broadcasted_iota(jnp.int32, (8, 128), 0)
        kf = [key_v[0:8, :], jnp.where(sub < nt - 8, key_v[8:16, :], 0.0)]
        cand = jnp.zeros((8, 128), F32)
        for i in range(C):
            mx = jnp.max(jnp.maximum(kf[0], kf[1]), axis=1, keepdims=True)
            mx = jnp.max(mx, axis=0, keepdims=True)
            kf = [jnp.where(k == mx, 0.0, k) for k in kf]
            cand = jnp.where(lane == i, mx, cand)
            if i == C - 1:
                cand_v[...] = cand
            yield _slab(cand)

    cp_wo.wait()
    cp_wd.wait()
    cp_wr.wait()
    if not MODB1:
        cp_wmb.wait()
    wds = _Pieces(wd_transpose())
    pre = _Pieces(preselect())
    queue = [_Pieces(mod_b())]
    dep = dep2 = None
    lag = 0
    for t in range(S // R3):
        att = None
        for kc in range(nkc):
            part = out_proj_chunk(t, kc, [dep, dep2])
            att = part if att is None else att + part
            dep = None
            while queue and dep is None:
                dep = queue[0].step()
                if dep is None:
                    queue.pop(0)
            dep2 = wds.step() if (1 <= t < 13 and kc % WDP == WDO) else None
            if t == S // R3 - 1:
                dep2 = pre.step()
        queue.append(_Pieces(epilogue(t, att)))
    wds.drain()
    pre.drain()
    for pcs in queue:
        pcs.drain()
    cp_out.start()

    lane_d = lax.broadcasted_iota(jnp.int32, (D, 128), 1)
    sub = lax.broadcasted_iota(jnp.int32, (8, 128), 0)
    sub16 = lax.broadcasted_iota(jnp.int32, (16, D), 0)
    sub8 = lax.broadcasted_iota(jnp.int32, (8, D), 0)
    rows_ = [cand_v[0:1, :]] + [key_v[t:t + 1, :] for t in range(S // R3 - NLATEKEYS, S // R3)]
    cols_ = [jnp.broadcast_to(a, (128, 128)).T for a in rows_]
    cols_[0] = cols_[0][0:C]
    best = jnp.zeros((8, 128), F32)
    for a in rows_:
        rank = None
        for ct in cols_:
            cnt = _vsum(jnp.where(ct > a, 1.0, 0.0))
            rank = cnt if rank is None else rank + cnt
        rank = jnp.sum(rank, axis=0, keepdims=True)
        best = jnp.maximum(best, jnp.where(rank == sub.astype(F32), a, 0.0))
    top = jnp.broadcast_to(jnp.max(best, axis=1, keepdims=True), (8, 128))
    mi = pltpu.bitcast(top, jnp.int32) - 0x00800000
    uu = jnp.right_shift(mi, 11) - 32768
    uu = jnp.where(uu < 0, uu ^ 0x7FFF, uu)
    r_sel = pltpu.bitcast(uu << 16, F32)
    tokv = (S - 1) - (mi & (S - 1))
    h_sel = jnp.zeros((8, D), F32)
    idxs = []
    for i in range(C):
        idx = tokv[i, 0]
        idxs.append(idx)
        b16 = pl.multiple_of((idx >> 4) << 4, 16)
        tile = h2r_v[pl.ds(b16, 16), 0:D].astype(F32)
        row = jnp.sum(jnp.where(sub16 == (idx & 15), tile, 0.0), axis=0, keepdims=True)
        h_sel = jnp.where(sub8 == i, row, h_sel)

    hb = _pad_rows(h_sel, 16).astype(BF)
    cp_wg.wait(); cp_wu.wait()
    gate = _b(jnp.dot(hb, wg_v[...], preferred_element_type=F32)[0:8])
    up = _b(jnp.dot(hb, wu_v[...], preferred_element_type=F32)[0:8])
    act = _pad_rows(_b(_b(gate * _sigmoid_b(gate)) * up), 16).astype(BF)
    xg = jnp.zeros((D, 128), BF)
    for i in range(C):
        t0 = pl.multiple_of((idxs[i] >> 7) << 7, 128)
        tile = pltpu.roll(x_v[:, pl.ds(t0, 128)], (i - (idxs[i] & 127)) & 127, 1)
        xg = jnp.where(lane_d == i, tile, xg)
    x1_t = _pad_rows(xg, 640).T
    x1_sel = x1_t[0:8, 0:D].astype(F32)
    wdn = _pin(wdn_v[...], [_join(x1_t[0:16, 0:128], x1_t[0:16, 512:640])], never, late=False) if PINX else wdn_v[...]
    y = _b(jnp.dot(act, wdn, preferred_element_type=F32)[0:8])
    y = _b(y * _lanes(_sigmoid_b(r_sel), 5)[:, 0:D])
    new = (x1_sel + _b(gbr_v[...] * _b(h_sel + y))).astype(BF)
    new_c = _pad_rows(new, 128)
    new_p = jnp.concatenate([new_c, jnp.zeros((128, 640 - D), BF)], axis=1).T[0:D]
    cp_out.wait()
    for i in range(C):
        idx = idxs[i]
        t0 = pl.multiple_of((idx >> 7) << 7, 128)
        rolled = pltpu.roll(new_p, ((idx & 127) - i) & 127, 1)
        out_v[:, pl.ds(t0, 128)] = jnp.where(lane_d == (idx & 127), rolled, out_v[:, pl.ds(t0, 128)])

    patches = []
    for i in range(C):
        ti = idxs[i] >> 7
        fresh = ti >= 0
        for j in range(i):
            fresh = jnp.logical_and(fresh, ti != (idxs[j] >> 7))
        t0 = pl.multiple_of(ti << 7, 128)
        cp = pltpu.make_async_copy(out_v.at[:, pl.ds(t0, 128)], out_hbm.at[0, :, pl.ds(t0, 128)],
                                   sems.at[PATCH_SEM + i])
        patches.append((fresh, cp))
        pl.when(fresh)(cp.start)
    for fresh, cp in patches:
        pl.when(fresh)(cp.wait)


@jax.jit
def pallas_adaLN_cond__gqa_block_cached__moe_arch_mod__prompt_kernel(
    A_x, A_k_cache, A_v_cache, A_wq, A_wo, B_x, B_w_r, B_w_gate, B_w_up, B_w_down, c, w_mod,
):
    del B_x
    any_spec = pl.BlockSpec(memory_space=pl.ANY)
    col = pltpu.VMEM((D, 128), F32)
    out_t = pl.pallas_call(
        _kernel,
        out_shape=jax.ShapeDtypeStruct((1, D, S), BF),
        in_specs=[any_spec] * 11 + [
                  pl.BlockSpec(memory_space=pltpu.SMEM)],
        out_specs=any_spec,
        scratch_shapes=[
            pltpu.VMEM((D, S), BF),
            pltpu.VMEM((HKV, SK, DH), BF),
            pltpu.VMEM((HKV, SK, DH), BF),
            pltpu.VMEM((D, HQ * DH), BF),
            pltpu.VMEM((D, HQ * DH), BF),
            pltpu.VMEM((D, F), BF),
            pltpu.VMEM((D, F), BF),
            pltpu.VMEM((D, F), BF),
            pltpu.VMEM((F, D), BF),
            pltpu.VMEM((D, 6 * D), BF),
            pltpu.VMEM((HQ, S, DH), BF),
            pltpu.VMEM((HQ + 1, S, DH), BF),
            pltpu.VMEM((D, S), BF),
            pltpu.VMEM((S, 640), BF),
            pltpu.VMEM((2, R1, 640), BF),
            pltpu.VMEM((1, D), BF),
            pltpu.VMEM((D,), BF),
            col, col, col, col, col, col, col,
            pltpu.VMEM((8, D), F32),
            pltpu.VMEM((16, 128), F32),
            pltpu.VMEM((8, 128), F32),
            pltpu.VMEM((RA, DH), F32),
            pltpu.VMEM((RA, 128), F32),
            pltpu.SemaphoreType.DMA((21 + C,)),
        ],
        compiler_params=pltpu.CompilerParams(vmem_limit_bytes=120 * 1024 * 1024),
        name="adaln_gqa_moe",
    )(jnp.swapaxes(A_x, 1, 2), A_k_cache, A_v_cache, A_wq, A_wo.T, B_w_r, B_w_gate, B_w_up, B_w_down.T, c, w_mod,
      np.zeros((1,), np.int32))
    return jnp.swapaxes(out_t, 1, 2)
```

```python
import numpy as np
import jax
import jax.numpy as jnp
from jax import lax
import jax.experimental.pallas as pl
import jax.experimental.pallas.tpu as pltpu

S = 2048
D = 576
HQ, HKV, DH = 32, 16, 128
SK = 2048
F = 4608
C = 8

BF = jnp.bfloat16
F32 = jnp.float32
U32 = jnp.uint32
NT = (((1,), (1,)), ((), ()))

LOG2E = 1.4426950408889634
QSCALE = (DH ** -0.5) * LOG2E
EPS_BF = 1.0013580322265625e-05

R1 = 256
RA = 128
CK = 512
R3 = 128
NQ = 512
KC = 512
UNROLLED1 = 5
XB = [0, 2 * R1, 3 * R1, S]
WB = [0, 512, 1536, 2560, 4096]


def _b(x):
    return x.astype(BF).astype(F32)


def _vsum(x):
    return jnp.sum(x.reshape(x.shape[0] // 8, 8, x.shape[1]), axis=0)


def _sigmoid_b(x):
    return _b(1.0 / _b(1.0 + _b(jnp.exp(-x))))


def _inv_std(sumsq):
    var = jnp.sum(sumsq, axis=0, keepdims=True) * (1.0 / D)
    return 1.0 / _b(jnp.sqrt(_b(_b(var) + EPS_BF)))


def _cols(row):
    return jnp.broadcast_to(row, (128, row.shape[1])).T


def _lanes(v, n):
    return jnp.concatenate([v] * n, axis=1) if n > 1 else v


def _pad_rows(x, n):
    if x.shape[0] == n:
        return x
    return jnp.concatenate([x, jnp.zeros((n - x.shape[0], x.shape[1]), x.dtype)], axis=0)


def _rows(bounds):
    return [slice(a, b) for a, b in zip(bounds[:-1], bounds[1:])]


def _slab(x):
    x = x[x.shape[0] - 8:, 0:128]
    return jnp.concatenate([x, x], axis=0).astype(BF)


def _fold(x):
    u = pltpu.bitcast(x, U32)
    acc = u[0:8]
    for i in range(1, u.shape[0] // 8):
        acc = acc | u[8 * i:8 * i + 8]
    return pltpu.bitcast(acc, BF)


def _join(a, b):
    return pltpu.bitcast(pltpu.bitcast(a, U32) | pltpu.bitcast(b, U32), BF)


def _late(d):
    return pltpu.bitcast(pltpu.roll(pltpu.bitcast(d, U32), 1, 1), BF)


def _pin(w, deps, never, late=True):
    if all(d is None for d in deps):
        return w
    deps = [None if d is None else (_late(d) if late else d) for d in deps]
    tops = []
    for i, d in enumerate(deps):
        t = w[0:16, i * 128:(i + 1) * 128]
        tops.append(t if d is None else jnp.where(never, d, t))
    if w.shape[1] > 128 * len(deps):
        tops.append(w[0:16, 128 * len(deps):])
    top = tops[0] if len(tops) == 1 else jnp.concatenate(tops, axis=1)
    return jnp.concatenate([top, w[16:]], axis=0)


class _Pieces:
    def __init__(self, gen):
        self.gen = gen

    def step(self, k=1):
        dep = None
        for _ in range(k):
            d = next(self.gen, None)
            dep = d if d is not None else dep
        return dep

    def drain(self):
        for _ in self.gen:
            pass


def _kernel(x_hbm, k_hbm, v_hbm, wq_hbm, wo_hbm, wr_hbm, wg_hbm, wu_hbm, wd_hbm, c_hbm, wm_hbm, zero_ref,
            out_hbm,
            x_v, k_v, v_v, wq_v, wo_v, wg_v, wu_v, wd_v, wdn_v, wm_v, q_v, o_v, out_v, h2r_v, h_v,
            c_v, wrin_v, sa_v, ca_v, ga_v, sb_v, cb_v, gb_v, wr_v, gbr_v, key_v, cand_v, acc_v, l_v, sems):
    never = zero_ref[0] != 0
    nx = S // R1
    nq = (HQ * DH) // NQ

    def colcopy(src, dst, lo, hi, sem):
        return pltpu.make_async_copy(src.at[:, pl.ds(lo, hi - lo)], dst.at[:, pl.ds(lo, hi - lo)], sems.at[sem])

    cp_wma = colcopy(wm_hbm, wm_v, 0, 2 * D, 0)
    cp_wmb = colcopy(wm_hbm, wm_v, 2 * D, 6 * D, 1)
    cp_x = [colcopy(x_hbm.at[0], x_v, XB[i], XB[i + 1], 2 + i) for i in range(len(XB) - 1)]
    cp_wq = [colcopy(wq_hbm, wq_v, WB[i], WB[i + 1], 6 + i) for i in range(len(WB) - 1)]
    cp_k = pltpu.make_async_copy(k_hbm.at[0], k_v, sems.at[12])
    cp_v = pltpu.make_async_copy(v_hbm.at[0], v_v, sems.at[13])
    cp_wo = pltpu.make_async_copy(wo_hbm, wo_v, sems.at[14])
    cp_wg = pltpu.make_async_copy(wg_hbm, wg_v, sems.at[15])
    cp_wu = pltpu.make_async_copy(wu_hbm, wu_v, sems.at[16])
    cp_wd = pltpu.make_async_copy(wd_hbm, wd_v, sems.at[17])
    cp_out = pltpu.make_async_copy(out_v, out_hbm.at[0], sems.at[18])
    cp_c = pltpu.make_async_copy(c_hbm, c_v, sems.at[19])
    cp_wr = pltpu.make_async_copy(wr_hbm, wrin_v, sems.at[20])
    patch_sem = 21

    cp_c.start()
    cp_wma.start()
    cp_x[0].start()
    cp_wq[0].start()
    cp_wr.start()

    cp_c.wait()
    c = c_v[...].astype(F32)
    sc = _b(c * _sigmoid_b(c)).astype(BF)
    sc8 = jnp.broadcast_to(sc, (8, D))
    cp_wma.wait()
    cp_wq[1].start()
    moda = _b(jnp.dot(sc8, wm_v[:, 0:2 * D], preferred_element_type=F32))[0:1]
    moda_c = _cols(moda)
    sa_v[...] = moda_c[0:D]
    ca_v[...] = _b(1.0 + moda_c[D:2 * D])

    KP = _rows([0, 128, 256, 384, 512, D])
    nl1 = R1 // 128

    def ln1(t):
        cols = pl.ds(pl.multiple_of(jnp.minimum(t, nx - 1) * R1, R1), R1)
        xs = [x_v[r, cols].astype(F32) for r in KP]
        tot = _vsum(xs[0])
        for xp in xs[1:]:
            tot = tot + _vsum(xp)
        yield _slab(tot)
        mean = jnp.sum(tot, axis=0, keepdims=True) * (1.0 / D)
        tot = None
        for xp in xs:
            xc = xp - mean
            tot = _vsum(xc * xc) if tot is None else tot + _vsum(xc * xc)
        yield _slab(tot)
        inv = _inv_std(tot)
        mean_b = _b(mean)
        for i, (r, xp) in enumerate(zip(KP, xs)):
            hn = _b(_b(xp - mean_b) * inv)
            hv = _b(hn * _lanes(ca_v[r, :], nl1)) + _lanes(sa_v[r, :], nl1)
            ht = _pad_rows(hv.astype(BF), 128).T
            h_v[t % 2, :, i * 128:(i + 1) * 128] = ht
            yield _fold(ht)

    def q_chunk(t, h, n, dep):
        rows = pl.ds(pl.multiple_of(t * R1, R1), R1)
        w = _pin(wq_v[:, n * NQ:(n + 1) * NQ], [dep], never)
        qn = jnp.dot(h, w, preferred_element_type=F32) * QSCALE
        for i in range(NQ // DH):
            q_v[n * (NQ // DH) + i, rows, :] = qn[:, i * DH:(i + 1) * DH].astype(BF)

    def q_tile(t):
        h = h_v[t % 2, :, 0:D]
        pcs = _Pieces(ln1(t + 1))
        dep = None
        for n in range(nq):
            q_chunk(t, h, n, dep)
            dep = pcs.step()
        pcs.drain()

    sweep = {0: ([cp_wq[0]], [cp_wq[2]]), 2: ([cp_wq[1]], [cp_wq[3]]), 6: ([cp_wq[2]], [cp_x[1]]),
             10: ([cp_wq[3], cp_x[1]], [cp_x[2]])}
    cp_x[0].wait()
    _Pieces(ln1(0)).drain()
    hs = [h_v[0, :, 0:D], None]
    for i in range(2 * nq):
        if i in sweep:
            for cp in sweep[i][0]:
                cp.wait()
            for cp in sweep[i][1]:
                cp.start()
        dep = None
        if i == 0:
            pcs = _Pieces(ln1(1))
        elif i == 1:
            dep = pcs.step(7)
            hs[1] = h_v[1, :, 0:D]
        elif i == 10:
            pcs = _Pieces(ln1(2))
        elif i > 10:
            dep = pcs.step(1 if i < 2 * nq - 1 else 7)
        q_chunk(i % 2, hs[i % 2], i // 2, dep)
    cp_x[2].wait()
    cp_k.start(); cp_v.start(); cp_wmb.start()
    for t in range(2, UNROLLED1):
        q_tile(t)

    def q_body(t, carry):
        q_tile(t)
        return carry

    lax.fori_loop(UNROLLED1, nx, q_body, 0)

    nck = SK // CK
    rep = HQ // HKV

    def finalize(acc, l, hq, t0):
        lsum = jnp.sum(l, axis=1, keepdims=True)
        rl = pl.reciprocal(lsum, approx=True)
        rl = rl * (2.0 - lsum * rl)
        ob = (acc * rl).astype(BF)
        o_v[hq, pl.ds(t0, RA), :] = ob
        return ob

    def attn_body(g, carry):
        tiles = [(hh, t) for hh in range(rep) for t in range(S // RA)]
        steps = [(ti, j) for ti in range(len(tiles)) for j in range(nck)]

        def qk(ti, j, dep=None):
            hh, t = tiles[ti]
            q = q_v[g * rep + hh, t * RA:(t + 1) * RA, :]
            return lax.dot_general(q, _pin(k_v[g, j * CK:(j + 1) * CK, :], [dep], never), NT,
                                   preferred_element_type=F32)

        s = qk(0, 0)
        prev_head = jnp.where(g == 0, HQ, g * rep - 1)
        dep = _fold(finalize(acc_v[...], l_v[...], prev_head, S - RA))
        m = l = acc = None
        for n, (ti, j) in enumerate(steps):
            s_next = None
            if n + 1 < len(steps):
                s_next = qk(*steps[n + 1], dep=dep if j == 2 else None)
            cm = s[:, 0:128]
            for i in range(1, CK // 128):
                cm = jnp.maximum(cm, s[:, i * 128:(i + 1) * 128])
            cm = jnp.max(cm, axis=1, keepdims=True)
            if m is None:
                m_new, alpha = cm, None
            else:
                m_new = jnp.maximum(m, cm)
                alpha = jnp.exp2(m - m_new)
            p = jnp.exp2(s - m_new)
            ls = p[:, 0:128]
            for i in range(1, CK // 128):
                ls = ls + p[:, i * 128:(i + 1) * 128]
            l = ls if l is None else alpha * l + ls
            o = jnp.dot(p.astype(BF), v_v[g, j * CK:(j + 1) * CK, :], preferred_element_type=F32)
            acc = o if acc is None else alpha * acc + o
            m = m_new
            if j == nck - 1:
                hh, t = tiles[ti]
                if ti + 1 < len(tiles):
                    dep = _fold(finalize(acc, l, g * rep + hh, t * RA))
                else:
                    acc_v[...] = acc
                    l_v[...] = l
                m = l = acc = None
            s = s_next
        return carry

    acc_v[...] = jnp.zeros((RA, DH), F32)
    l_v[...] = jnp.ones((RA, 128), F32)
    cp_k.wait()
    cp_v.wait()
    cp_wo.start(); cp_wd.start(); cp_wg.start(); cp_wu.start()
    lax.fori_loop(0, HKV, attn_body, 0)
    finalize(acc_v[...], l_v[...], HQ - 1, S - RA)

    lane = lax.broadcasted_iota(jnp.int32, (8, 128), 1)
    nkc = HQ * DH // KC
    nt3 = S // R3
    n_late = 2

    def mod_b():
        for i, (dst, plus1) in enumerate([(ga_v, False), (sb_v, False), (cb_v, True), (gb_v, False)]):
            if i % 2 == 0:
                modb = _b(jnp.dot(sc8, wm_v[:, (2 + i) * D:(4 + i) * D], preferred_element_type=F32))
                modb_c = _cols(modb[0:1])
            val = modb_c[(i % 2) * D:(i % 2 + 1) * D]
            val = _b(1.0 + val) if plus1 else val
            dst[...] = val
            if i == 3:
                gbr_v[...] = modb[:, D:2 * D]
            yield _slab(val)
        val = _cols(wrin_v[...].astype(F32).reshape(1, D))
        wr_v[...] = val
        yield _slab(val)

    def out_proj_chunk(t, kc, deps):
        cols = slice(t * R3, (t + 1) * R3)
        hpc = KC // DH
        ocat = jnp.concatenate([o_v[kc * hpc + i, cols, :] for i in range(hpc)], axis=1)
        return lax.dot_general(wo_v[:, kc * KC:(kc + 1) * KC], _pin(ocat, deps, never), NT,
                               preferred_element_type=F32)

    def epilogue(t, att):
        cols = slice(t * R3, (t + 1) * R3)
        tot = None
        for r in _rows([0, D // 2, D]):
            x1 = _b(x_v[r, cols].astype(F32) + _b(ga_v[r, :] * _b(att[r])))
            x_v[r, cols] = x1.astype(BF)
            tot = _vsum(x1) if tot is None else tot + _vsum(x1)
            yield _slab(tot)
        mean = jnp.sum(tot, axis=0, keepdims=True) * (1.0 / D)
        tot = None
        for i, r in enumerate(KP):
            xc = x_v[r, cols].astype(F32) - mean
            tot = _vsum(xc * xc) if tot is None else tot + _vsum(xc * xc)
            if i == 1:
                yield _slab(tot)
        yield _slab(tot)
        inv = _inv_std(tot)
        mean_b = _b(mean)
        rs = None
        for i, r in enumerate(KP):
            xp = x_v[r, cols].astype(F32)
            hn = _b(_b(xp - mean_b) * inv)
            h2b = (_b(hn * cb_v[r, :]) + sb_v[r, :]).astype(BF)
            h2 = h2b.astype(F32)
            out_v[r, cols] = (xp + _b(gb_v[r, :] * h2)).astype(BF)
            rp = _vsum(h2 * wr_v[r, :])
            rs = rp if rs is None else rs + rp
            h2t = _pad_rows(h2b, 128).T
            h2r_v[cols, i * 128:(i + 1) * 128] = h2t
            d = _join(_slab(rs), _fold(h2t))
            dep = d if i != len(KP) - 1 else _join(dep, d)
            if i < 3:
                yield dep
        r = _b(jnp.sum(rs, axis=0, keepdims=True))
        rb = pltpu.bitcast(jnp.broadcast_to(r, (8, 128)), jnp.int32)
        u = jnp.right_shift(rb, 16)
        u = jnp.where(u < 0, u ^ 0x7FFF, u) + 32768
        tok = t * 128 + lane
        kb = (u << 11) + (S - 1 - tok) + 0x00800000
        key_v[t:t + 1, :] = pltpu.bitcast(kb, F32)[0:1]
        yield dep

    def wd_transpose():
        for j in range(F // 128):
            blk = _pad_rows(wd_v[:, j * 128:(j + 1) * 128], 640).T[:, 0:D]
            wdn_v[j * 128:(j + 1) * 128, :] = blk
            dep = _fold(blk[:, 0:128])
            for i in range(1, 4):
                dep = _join(dep, _fold(blk[:, i * 128:(i + 1) * 128]))
            yield _join(dep, blk[112:128, 448:D])

    def preselect():
        sub = lax.broadcasted_iota(jnp.int32, (8, 128), 0)
        kf = [key_v[0:8, :], jnp.where(sub < nt3 - n_late - 8, key_v[8:16, :], 0.0)]
        cand = jnp.zeros((8, 128), F32)
        for i in range(C):
            mx = jnp.max(jnp.maximum(kf[0], kf[1]), axis=1, keepdims=True)
            mx = jnp.max(mx, axis=0, keepdims=True)
            kf = [jnp.where(k == mx, 0.0, k) for k in kf]
            cand = jnp.where(lane == i, mx, cand)
            if i == C - 1:
                cand_v[...] = cand
            yield _slab(cand)

    cp_wo.wait()
    cp_wd.wait()
    cp_wr.wait()
    cp_wmb.wait()
    wds = _Pieces(wd_transpose())
    pre = _Pieces(preselect())
    queue = [_Pieces(mod_b())]
    dep = dep2 = held = None
    for t in range(nt3):
        att = None
        for kc in range(nkc):
            part = out_proj_chunk(t, kc, [dep, dep2])
            att = part if att is None else att + part
            dep = None
            while queue and dep is None:
                dep = queue[0].step()
                if dep is None:
                    queue.pop(0)
            if t == 0:
                dep, held = held, dep
            dep2 = wds.step() if (1 <= t < 13 and kc % 3 == 2) else None
            if t == nt3 - 1:
                dep2 = pre.step()
        queue.append(_Pieces(epilogue(t, att)))
    wds.drain()
    pre.drain()
    for pcs in queue:
        pcs.drain()
    cp_out.start()

    lane_d = lax.broadcasted_iota(jnp.int32, (D, 128), 1)
    sub = lax.broadcasted_iota(jnp.int32, (8, 128), 0)
    sub16 = lax.broadcasted_iota(jnp.int32, (16, D), 0)
    sub8 = lax.broadcasted_iota(jnp.int32, (8, D), 0)
    rows_ = [cand_v[0:1, :]] + [key_v[t:t + 1, :] for t in range(nt3 - n_late, nt3)]
    cols_ = [jnp.broadcast_to(a, (128, 128)).T for a in rows_]
    cols_[0] = cols_[0][0:C]
    best = jnp.zeros((8, 128), F32)
    for a in rows_:
        rank = None
        for ct in cols_:
            cnt = _vsum(jnp.where(ct > a, 1.0, 0.0))
            rank = cnt if rank is None else rank + cnt
        rank = jnp.sum(rank, axis=0, keepdims=True)
        best = jnp.maximum(best, jnp.where(rank == sub.astype(F32), a, 0.0))
    top = jnp.broadcast_to(jnp.max(best, axis=1, keepdims=True), (8, 128))
    mi = pltpu.bitcast(top, jnp.int32) - 0x00800000
    uu = jnp.right_shift(mi, 11) - 32768
    uu = jnp.where(uu < 0, uu ^ 0x7FFF, uu)
    r_sel = pltpu.bitcast(uu << 16, F32)
    tokv = (S - 1) - (mi & (S - 1))
    h_sel = jnp.zeros((8, D), F32)
    idxs = []
    for i in range(C):
        idx = tokv[i, 0]
        idxs.append(idx)
        b16 = pl.multiple_of((idx >> 4) << 4, 16)
        tile = h2r_v[pl.ds(b16, 16), 0:D].astype(F32)
        row = jnp.sum(jnp.where(sub16 == (idx & 15), tile, 0.0), axis=0, keepdims=True)
        h_sel = jnp.where(sub8 == i, row, h_sel)

    hb = _pad_rows(h_sel, 16).astype(BF)
    cp_wg.wait(); cp_wu.wait()
    gate = _b(jnp.dot(hb, wg_v[...], preferred_element_type=F32)[0:8])
    up = _b(jnp.dot(hb, wu_v[...], preferred_element_type=F32)[0:8])
    act = _pad_rows(_b(_b(gate * _sigmoid_b(gate)) * up), 16).astype(BF)
    xg = jnp.zeros((D, 128), BF)
    for i in range(C):
        t0 = pl.multiple_of((idxs[i] >> 7) << 7, 128)
        tile = pltpu.roll(x_v[:, pl.ds(t0, 128)], (i - (idxs[i] & 127)) & 127, 1)
        xg = jnp.where(lane_d == i, tile, xg)
    x1_t = _pad_rows(xg, 640).T
    x1_sel = x1_t[0:8, 0:D].astype(F32)
    wdn = _pin(wdn_v[...], [_join(x1_t[0:16, 0:128], x1_t[0:16, 512:640])], never, late=False)
    y = _b(jnp.dot(act, wdn, preferred_element_type=F32)[0:8])
    y = _b(y * _lanes(_sigmoid_b(r_sel), 5)[:, 0:D])
    new = (x1_sel + _b(gbr_v[...] * _b(h_sel + y))).astype(BF)
    new_c = _pad_rows(new, 128)
    new_c = jnp.concatenate([new_c, jnp.zeros((128, 640 - D), BF)], axis=1).T[0:D]
    cp_out.wait()
    for i in range(C):
        idx = idxs[i]
        t0 = pl.multiple_of((idx >> 7) << 7, 128)
        rolled = pltpu.roll(new_c, ((idx & 127) - i) & 127, 1)
        out_v[:, pl.ds(t0, 128)] = jnp.where(lane_d == (idx & 127), rolled, out_v[:, pl.ds(t0, 128)])

    patches = []
    for i in range(C):
        ti = idxs[i] >> 7
        fresh = ti >= 0
        for j in range(i):
            fresh = jnp.logical_and(fresh, ti != (idxs[j] >> 7))
        t0 = pl.multiple_of(ti << 7, 128)
        cp = pltpu.make_async_copy(out_v.at[:, pl.ds(t0, 128)], out_hbm.at[0, :, pl.ds(t0, 128)],
                                   sems.at[patch_sem + i])
        patches.append((fresh, cp))
        pl.when(fresh)(cp.start)
    for fresh, cp in patches:
        pl.when(fresh)(cp.wait)


@jax.jit
def pallas_adaLN_cond__gqa_block_cached__moe_arch_mod__prompt_kernel(
    A_x: jax.Array,
    A_k_cache: jax.Array,
    A_v_cache: jax.Array,
    A_wq: jax.Array,
    A_wo: jax.Array,
    B_x: jax.Array,
    B_w_r: jax.Array,
    B_w_gate: jax.Array,
    B_w_up: jax.Array,
    B_w_down: jax.Array,
    c: jax.Array,
    w_mod: jax.Array,
):
    del B_x
    any_spec = pl.BlockSpec(memory_space=pl.ANY)
    col = pltpu.VMEM((D, 128), F32)
    out_t = pl.pallas_call(
        _kernel,
        out_shape=jax.ShapeDtypeStruct((1, D, S), BF),
        in_specs=[any_spec] * 11 + [pl.BlockSpec(memory_space=pltpu.SMEM)],
        out_specs=any_spec,
        scratch_shapes=[
            pltpu.VMEM((D, S), BF),
            pltpu.VMEM((HKV, SK, DH), BF),
            pltpu.VMEM((HKV, SK, DH), BF),
            pltpu.VMEM((D, HQ * DH), BF),
            pltpu.VMEM((D, HQ * DH), BF),
            pltpu.VMEM((D, F), BF),
            pltpu.VMEM((D, F), BF),
            pltpu.VMEM((D, F), BF),
            pltpu.VMEM((F, D), BF),
            pltpu.VMEM((D, 6 * D), BF),
            pltpu.VMEM((HQ, S, DH), BF),
            pltpu.VMEM((HQ + 1, S, DH), BF),
            pltpu.VMEM((D, S), BF),
            pltpu.VMEM((S, 640), BF),
            pltpu.VMEM((2, R1, 640), BF),
            pltpu.VMEM((1, D), BF),
            pltpu.VMEM((D,), BF),
            col, col, col, col, col, col, col,
            pltpu.VMEM((8, D), F32),
            pltpu.VMEM((16, 128), F32),
            pltpu.VMEM((8, 128), F32),
            pltpu.VMEM((RA, DH), F32),
            pltpu.VMEM((RA, 128), F32),
            pltpu.SemaphoreType.DMA((21 + C,)),
        ],
        compiler_params=pltpu.CompilerParams(vmem_limit_bytes=120 * 1024 * 1024),
        name="adaln_gqa_moe",
    )(jnp.swapaxes(A_x, 1, 2), A_k_cache, A_v_cache, A_wq, A_wo.T, B_w_r, B_w_gate, B_w_up, B_w_down.T, c, w_mod,
      np.zeros((1,), np.int32))
    return jnp.swapaxes(out_t, 1, 2)
```
